```python
import jax
import jax.numpy as jnp

def _softmax(x, axis=-1):
    return jax.nn.softmax(x, axis=axis)
def _gelu(x):
    return jax.nn.gelu(x, approximate=True)
def _silu(x):
    return jax.nn.silu(x)
def _sigmoid(x):
    return jax.nn.sigmoid(x)
def _layernorm(x, axis=-1, eps=1e-5):
    m = jnp.mean(x, axis=axis, keepdims=True)
    v = jnp.var(x, axis=axis, keepdims=True)
    return (x - m) / jnp.sqrt(v + eps)
def _scatter_add(tgt, idx, src, axis=0):
    return tgt.at[idx].add(src)
def _segment_sum(src, seg, n):
    return jax.ops.segment_sum(src, seg, n)
class _Rng:
    def __init__(self, key):
        self._k = key
    def _next(self):
        self._k, sub = jax.random.split(self._k)
        return sub
    def normal(self, shape):
        return jax.random.normal(self._next(), shape, dtype=jnp.bfloat16)
    def randint(self, lo, hi, shape):
        return jax.random.randint(self._next(), shape, lo, hi, dtype=jnp.int32)
    def uniform(self, shape, lo=0.0, hi=1.0):
        return jax.random.uniform(self._next(), shape, jnp.bfloat16, lo, hi)
    def permutation(self, n):
        return jax.random.permutation(self._next(), n)


kernel_name = 'interleave_layers__sliding_block_cached__dense_activation_gelu__decode'

def _fwd_setup_inputs():
    _rng = _Rng(jax.random.key(int.from_bytes(__import__("os").urandom(4), "little")))
    _w = (lambda a: (lambda t: t.astype(jnp.bfloat16) if jnp.issubdtype(t.dtype, jnp.floating) else t)(jnp.asarray(a)))
    def _A_setup():
        B, Sq, D = 2, 1, 512
        Hq, Hkv, Sk, Dh = 32, 8, 32768, 128
        assert Hq % Hkv == 0, (Hq, Hkv)
        return {
            "x": _w((lambda *s: _rng.normal(s) * 0.05)(B, Sq, D)),
            "k_cache": _w((lambda *s: _rng.normal(s) * 0.05)(B, Hkv, Sk, Dh)),
            "v_cache": _w((lambda *s: _rng.normal(s) * 0.05)(B, Hkv, Sk, Dh)),
            "wq": _w((lambda *s: _rng.normal(s) * 0.05)(D, Hq * Dh) * (D ** -0.5)),
            "wo": _w((lambda *s: _rng.normal(s) * 0.05)(Hq * Dh, D) * ((Hq * Dh) ** -0.5)),
        }
    _A_in = _A_setup()

    def _B_setup():
        B, S, D, F = 2, 1, 512, 1792
        return {
            "x": _w((lambda *s: _rng.normal(s) * 0.05)(B, S, D)),
            "w1": _w((lambda *s: _rng.normal(s) * 0.05)(D, F) * (D ** -0.5)),
            "b1": _w((lambda *s: _rng.normal(s) * 0.05)(F) * 0.01),
            "w2": _w((lambda *s: _rng.normal(s) * 0.05)(F, D) * (F ** -0.5)),
            "b2": _w((lambda *s: _rng.normal(s) * 0.05)(D) * 0.01),
        }
    _B_in = _B_setup()

    return {
        "A_x": _A_in["x"],
        "A_k_cache": _A_in["k_cache"],
        "A_v_cache": _A_in["v_cache"],
        "A_wq": _A_in["wq"],
        "A_wo": _A_in["wo"],
        "B_x": _B_in["x"],
        "B_w1": _B_in["w1"],
        "B_b1": _B_in["b1"],
        "B_w2": _B_in["w2"],
        "B_b2": _B_in["b2"],
    }

def _fwd_reference(A_x, A_k_cache, A_v_cache, A_wq, A_wo, B_x, B_w1, B_b1, B_w2, B_b2):
    def _A_ref(x, k_cache, v_cache, wq, wo):
        B, Sq, D = x.shape
        Hq, Dh = 32, 128
        Hkv, Sk = k_cache.shape[1], k_cache.shape[2]
        W = min(4096, max(256, Sk // 4))
        rep = Hq // Hkv
        q = (lambda x, *d: x.transpose(*d))((x @ wq).reshape(B, Sq, Hq, Dh), 0, 2, 1, 3)
        k = jnp.repeat(k_cache[:, :, Sk - W:, :], rep, axis=1)
        v = jnp.repeat(v_cache[:, :, Sk - W:, :], rep, axis=1)
        scores = jnp.einsum("bhqd,bhkd->bhqk", q, k) * (Dh ** -0.5)
        p = _softmax(scores, axis=-1)
        o = jnp.einsum("bhqk,bhkd->bhqd", p, v)
        return (lambda x, *d: x.transpose(*d))(o, 0, 2, 1, 3).reshape(B, Sq, Hq * Dh) @ wo

    def _B_ref(x, w1, b1, w2, b2):
        h = jnp.einsum("bsd,df->bsf", x, w1) + b1
        h = _gelu(h)
        return jnp.einsum("bsf,fd->bsd", h, w2) + b2

    x = A_x
    x = x + _A_ref(_layernorm(x, axis=-1), A_k_cache, A_v_cache, A_wq, A_wo)
    x = x + _B_ref(_layernorm(x, axis=-1), B_w1, B_b1, B_w2, B_b2)
    x = x + _A_ref(_layernorm(x, axis=-1), A_k_cache, A_v_cache, A_wq, A_wo)
    x = x + _B_ref(_layernorm(x, axis=-1), B_w1, B_b1, B_w2, B_b2)
    return x


def setup_inputs():
    _inp = _fwd_setup_inputs()
    _gk = jax.random.fold_in(jax.random.key(int.from_bytes(__import__("os").urandom(4), "little")), 2**31 - 1)
    _shapes = [[2, 1, 512]]
    _dtypes = ['bfloat16']
    _gks = jax.random.split(_gk, len(_shapes))
    _gs = [jax.random.normal(k, s, dtype=jnp.dtype(d)) * 0.05 for k, s, d in zip(_gks, _shapes, _dtypes)]
    _inp["grad_out"] = _gs[0]
    return _inp

def reference(A_x, A_k_cache, A_v_cache, A_wq, A_wo, B_w1, B_b1, B_w2, B_b2, B_x, grad_out):
    _const = dict(B_x=B_x)
    def _f(*_d):
        return _fwd_reference(**{'A_x': _d[0], 'A_k_cache': _d[1], 'A_v_cache': _d[2], 'A_wq': _d[3], 'A_wo': _d[4], 'B_w1': _d[5], 'B_b1': _d[6], 'B_w2': _d[7], 'B_b2': _d[8], **_const})
    _out, _vjp = jax.vjp(_f, A_x, A_k_cache, A_v_cache, A_wq, A_wo, B_w1, B_b1, B_w2, B_b2)
    _grads = _vjp(grad_out)
    _out0 = jnp.asarray(_out)
    return (_out0, *[jnp.asarray(_g) for _g in _grads])
```

```python
import math

import jax
import jax.numpy as jnp
from jax import lax
import jax.experimental.pallas as pl
import jax.experimental.pallas.tpu as pltpu

_F32 = jnp.float32
_BF16 = jnp.bfloat16
_NT = (((1,), (1,)), ((), ()))


def _dot(a, b):
    return jnp.dot(a, b, preferred_element_type=_F32)


def _dot_nt(a, b):
    return lax.dot_general(a, b, _NT, preferred_element_type=_F32)


def _ln_fwd(x):
    m = jnp.mean(x, axis=-1, keepdims=True)
    xc = x - m
    var = jnp.mean(xc * xc, axis=-1, keepdims=True)
    rstd = lax.rsqrt(var + 1e-5)
    return xc * rstd, rstd


def _ln_bwd(dxn, xn, rstd):
    m1 = jnp.mean(dxn, axis=-1, keepdims=True)
    m2 = jnp.mean(dxn * xn, axis=-1, keepdims=True)
    return rstd * (dxn - m1 - xn * m2)


_GELU_C = math.sqrt(2.0 / math.pi)


def _gelu_and_grad(x):
    x2 = x * x
    t = jnp.tanh(_GELU_C * (x + 0.044715 * x2 * x))
    y = 0.5 * x * (1.0 + t)
    dy = 0.5 * (1.0 + t) + 0.5 * x * (1.0 - t * t) * _GELU_C * (1.0 + 3.0 * 0.044715 * x2)
    return y, dy


@jax.jit
def pallas_interleave_layers__sliding_block_cached__dense_activation_gelu__decode_kernel(
    A_x: jax.Array,
    A_k_cache: jax.Array,
    A_v_cache: jax.Array,
    A_wq: jax.Array,
    A_wo: jax.Array,
    B_x: jax.Array,
    B_w1: jax.Array,
    B_b1: jax.Array,
    B_w2: jax.Array,
    B_b2: jax.Array,
    grad_out: jax.Array,
):
    B, Sq, D = A_x.shape
    _, Hkv, Sk, Dh = A_k_cache.shape
    HD = A_wq.shape[1]
    Hq = HD // Dh
    F = B_w1.shape[1]
    W = min(4096, max(256, Sk // 4))
    rep = Hq // Hkv
    assert Sq == 1 and B == 2 and rep == 4 and Dh == 128 and Hq == 32
    G = B * Hkv
    R = G * 8
    assert R == 128
    Z = Sk - W
    scale = Dh ** -0.5

    def kernel(x_ref, k_hbm, v_hbm, wq_hbm, wo_hbm, w1_hbm, b1_ref, w2_hbm, b2_ref, go_ref,
               out_ref, gx_ref, gk_hbm, gv_hbm, gwq_hbm, gwo_hbm, gw1_hbm, gb1_ref, gw2_hbm, gb2_ref,
               kb, vb, wq_v, wo_v, w1_v, w2_v, gwq_v, gwo_v, gw1_v, gw2_v, z_ref,
               p_all, ds_all, pt_ref, dst_ref, q_all, o_all, do_all, dq_all,
               row_ref, flat_ref,
               xa_p, dq_p, o_p, ga_p, xb_p, dh_p, h_p, gb_p,
               ksem, vsem, wsem, zsem, osem, gsem):
        def k_load(g):
            return pltpu.make_async_copy(
                k_hbm.at[g // Hkv, g % Hkv, pl.ds(Z, W), :], kb.at[g], ksem.at[g])

        def v_load(g):
            return pltpu.make_async_copy(
                v_hbm.at[g // Hkv, g % Hkv, pl.ds(Z, W), :], vb.at[g], vsem.at[g])

        w_loads = [
            pltpu.make_async_copy(wq_hbm, wq_v, wsem.at[0]),
            pltpu.make_async_copy(wo_hbm, wo_v, wsem.at[1]),
            pltpu.make_async_copy(w1_hbm, w1_v, wsem.at[2]),
            pltpu.make_async_copy(w2_hbm, w2_v, wsem.at[3]),
        ]
        w_loads[0].start()
        for g in range(G):
            k_load(g).start()
        for g in range(G):
            v_load(g).start()
        w_loads[1].start()
        w_loads[2].start()
        w_loads[3].start()

        z_ref[...] = jnp.zeros(z_ref.shape, z_ref.dtype)
        z_copies = []
        for dst in (gk_hbm, gv_hbm):
            for g in range(G):
                cp = pltpu.make_async_copy(
                    z_ref, dst.at[g // Hkv, g % Hkv, pl.ds(0, Z), :], zsem.at[0])
                cp.start()
                z_copies.append(cp)

        q_all[...] = jnp.zeros(q_all.shape, _F32)
        do_all[...] = jnp.zeros(do_all.shape, _F32)
        for r in (xa_p, o_p, xb_p, h_p):
            r[...] = jnp.zeros(r.shape, r.dtype)
        for r in (dq_p, ga_p, dh_p, gb_p):
            r[...] = jnp.zeros(r.shape, r.dtype)

        def pad8(ref_2d):
            row_ref[...] = jnp.zeros(row_ref.shape, _F32)
            row_ref[0:B, :] = ref_2d[...].astype(_F32)
            return row_ref[...]

        def flat_to_rows(flat, tbl, layer):
            flat_ref[...] = flat
            for b in range(B):
                for h in range(Hq):
                    r = (b * Hkv + h // rep) * 8 + layer * rep + h % rep
                    tbl[r:r + 1, :] = flat_ref[b:b + 1, h * Dh:(h + 1) * Dh]

        def rows_to_flat(tbl, layer):
            flat_ref[...] = jnp.zeros(flat_ref.shape, _F32)
            for b in range(B):
                for h in range(Hq):
                    r = (b * Hkv + h // rep) * 8 + layer * rep + h % rep
                    flat_ref[b:b + 1, h * Dh:(h + 1) * Dh] = tbl[r:r + 1, :]
            return flat_ref[...]

        def attn_fwd(x, layer):
            xn, rstd = _ln_fwd(x)
            xa_p[layer * B:(layer + 1) * B, :] = xn[0:B, :]
            q = _dot(xn.astype(_BF16), wq_v[...])
            flat_to_rows(q.astype(_BF16).astype(_F32), q_all, layer)

            def body(g, c):
                r0 = pl.multiple_of(g * 8, 8)
                qg = q_all[pl.ds(r0, 8), :].astype(_BF16)
                s = _dot_nt(qg, kb[g]) * scale
                m = jnp.max(s, axis=-1, keepdims=True)
                e = jnp.exp(s - m)
                p = e / jnp.sum(e, axis=-1, keepdims=True)
                p_all[pl.ds(r0, 8), :] = p
                o_all[pl.ds(r0, 8), :] = _dot(p.astype(_BF16), vb[g])
                return c

            lax.fori_loop(0, G, body, 0)
            o = rows_to_flat(o_all, layer)
            o_p[layer * B:(layer + 1) * B, :] = o[0:B, :]
            y = _dot(o.astype(_BF16), wo_v[...])
            return x + y, xn, rstd

        def attn_bwd(gy, layer, xn, rstd):
            gyb = gy.astype(_BF16)
            ga_p[layer * B:(layer + 1) * B, :] = gyb[0:B, :]
            do = _dot_nt(gyb, wo_v[...])
            flat_to_rows(do, do_all, layer)

            def body(g, c):
                r0 = pl.multiple_of(g * 8, 8)
                dog = do_all[pl.ds(r0, 8), :].astype(_BF16)
                dp = _dot_nt(dog, vb[g])
                p = p_all[pl.ds(r0, 8), :]
                ds = p * (dp - jnp.sum(p * dp, axis=-1, keepdims=True)) * scale
                ds_all[pl.ds(r0, 8), :] = ds
                dq_all[pl.ds(r0, 8), :] = _dot(ds.astype(_BF16), kb[g])
                return c

            lax.fori_loop(0, G, body, 0)
            dq = rows_to_flat(dq_all, layer).astype(_BF16)
            dq_p[layer * B:(layer + 1) * B, :] = dq[0:B, :]
            dxn = _dot_nt(dq, wq_v[...])
            return gy + _ln_bwd(dxn, xn, rstd)

        def ffn_fwd(x, layer):
            xn, rstd = _ln_fwd(x)
            xb_p[layer * B:(layer + 1) * B, :] = xn[0:B, :]
            hpre = _dot(xn.astype(_BF16), w1_v[...]) + b1_ref[...].astype(_F32)
            h, dgelu = _gelu_and_grad(hpre)
            h_p[layer * B:(layer + 1) * B, :] = h[0:B, :]
            y = _dot(h.astype(_BF16), w2_v[...]) + b2_ref[...].astype(_F32)
            return x + y, xn, rstd, dgelu

        def ffn_bwd(gy, layer, xn, rstd, dgelu):
            gyb = gy.astype(_BF16)
            gb_p[layer * B:(layer + 1) * B, :] = gyb[0:B, :]
            dh = _dot_nt(gyb, w2_v[...])
            dhpre = dh * dgelu
            dhb = dhpre.astype(_BF16)
            dh_p[layer * B:(layer + 1) * B, :] = dhb[0:B, :]
            dxn = _dot_nt(dhb, w1_v[...])
            db1 = jnp.sum(dhpre[0:B, :], axis=0, keepdims=True)
            db2 = jnp.sum(gy[0:B, :], axis=0, keepdims=True)
            return gy + _ln_bwd(dxn, xn, rstd), db1, db2

        x0 = pad8(x_ref)
        w_loads[0].wait()
        for g in range(G):
            k_load(g).wait()
        for g in range(G):
            v_load(g).wait()
        w_loads[1].wait()
        x1, xn_a0, rs_a0 = attn_fwd(x0, 0)
        w_loads[2].wait()
        w_loads[3].wait()
        x2, xn_b0, rs_b0, dg0 = ffn_fwd(x1, 0)
        x3, xn_a1, rs_a1 = attn_fwd(x2, 1)
        x4, xn_b1, rs_b1, dg1 = ffn_fwd(x3, 1)
        out_ref[...] = x4[0:B, :].astype(out_ref.dtype)

        g4 = pad8(go_ref)
        g3, db1_1, db2_1 = ffn_bwd(g4, 1, xn_b1, rs_b1, dg1)
        g2 = attn_bwd(g3, 1, xn_a1, rs_a1)
        g1, db1_0, db2_0 = ffn_bwd(g2, 0, xn_b0, rs_b0, dg0)
        g0 = attn_bwd(g1, 0, xn_a0, rs_a0)
        gx_ref[...] = g0[0:B, :].astype(gx_ref.dtype)
        gb1_ref[...] = (db1_0 + db1_1).astype(gb1_ref.dtype)
        gb2_ref[...] = (db2_0 + db2_1).astype(gb2_ref.dtype)

        out_copies = []
        for i, (lhs, rhs, stage, dst) in enumerate((
                (xa_p, dq_p, gwq_v, gwq_hbm), (o_p, ga_p, gwo_v, gwo_hbm),
                (xb_p, dh_p, gw1_v, gw1_hbm), (h_p, gb_p, gw2_v, gw2_hbm))):
            lt = lhs[...].T.astype(_BF16)
            stage[...] = _dot(lt, rhs[...]).astype(_BF16)
            cp = pltpu.make_async_copy(stage, dst, gsem.at[i])
            cp.start()
            out_copies.append(cp)

        pt_ref[...] = p_all[...].T.astype(_BF16)
        dst_ref[...] = ds_all[...].T.astype(_BF16)
        rgrp = lax.broadcasted_iota(jnp.int32, (R, Dh), 0) // 8
        qv = q_all[...]
        dov = do_all[...]
        for g in range(G):
            qm = jnp.where(rgrp == g, qv, 0.0).astype(_BF16)
            kb[g] = _dot(dst_ref[...], qm).astype(_BF16)
            cp = pltpu.make_async_copy(
                kb.at[g], gk_hbm.at[g // Hkv, g % Hkv, pl.ds(Z, W), :], osem.at[0])
            cp.start()
            out_copies.append(cp)
            dm = jnp.where(rgrp == g, dov, 0.0).astype(_BF16)
            vb[g] = _dot(pt_ref[...], dm).astype(_BF16)
            cp = pltpu.make_async_copy(
                vb.at[g], gv_hbm.at[g // Hkv, g % Hkv, pl.ds(Z, W), :], osem.at[0])
            cp.start()
            out_copies.append(cp)

        for cp in z_copies:
            cp.wait()
        for cp in out_copies:
            cp.wait()

    vmem = pl.BlockSpec(memory_space=pltpu.VMEM)
    hbm = pl.BlockSpec(memory_space=pl.ANY)
    outs = pl.pallas_call(
        kernel,
        in_specs=[vmem, hbm, hbm, hbm, hbm, hbm, vmem, hbm, vmem, vmem],
        out_specs=[vmem, vmem, hbm, hbm, hbm, hbm, hbm, vmem, hbm, vmem],
        out_shape=[
            jax.ShapeDtypeStruct((B, D), _BF16),
            jax.ShapeDtypeStruct((B, D), _BF16),
            jax.ShapeDtypeStruct(A_k_cache.shape, _BF16),
            jax.ShapeDtypeStruct(A_v_cache.shape, _BF16),
            jax.ShapeDtypeStruct(A_wq.shape, _BF16),
            jax.ShapeDtypeStruct(A_wo.shape, _BF16),
            jax.ShapeDtypeStruct(B_w1.shape, _BF16),
            jax.ShapeDtypeStruct((1, F), _BF16),
            jax.ShapeDtypeStruct(B_w2.shape, _BF16),
            jax.ShapeDtypeStruct((1, D), _BF16),
        ],
        scratch_shapes=[
            pltpu.VMEM((G, W, Dh), _BF16),
            pltpu.VMEM((G, W, Dh), _BF16),
            pltpu.VMEM((D, HD), _BF16),
            pltpu.VMEM((HD, D), _BF16),
            pltpu.VMEM((D, F), _BF16),
            pltpu.VMEM((F, D), _BF16),
            pltpu.VMEM((D, HD), _BF16),
            pltpu.VMEM((HD, D), _BF16),
            pltpu.VMEM((D, F), _BF16),
            pltpu.VMEM((F, D), _BF16),
            pltpu.VMEM((Z, Dh), _BF16),
            pltpu.VMEM((R, W), _F32),
            pltpu.VMEM((R, W), _F32),
            pltpu.VMEM((W, R), _BF16),
            pltpu.VMEM((W, R), _BF16),
            pltpu.VMEM((R, Dh), _F32),
            pltpu.VMEM((R, Dh), _F32),
            pltpu.VMEM((R, Dh), _F32),
            pltpu.VMEM((R, Dh), _F32),
            pltpu.VMEM((8, D), _F32),
            pltpu.VMEM((8, HD), _F32),
            pltpu.VMEM((128, D), _F32),
            pltpu.VMEM((128, HD), _BF16),
            pltpu.VMEM((128, HD), _F32),
            pltpu.VMEM((128, D), _BF16),
            pltpu.VMEM((128, D), _F32),
            pltpu.VMEM((128, F), _BF16),
            pltpu.VMEM((128, F), _F32),
            pltpu.VMEM((128, D), _BF16),
            pltpu.SemaphoreType.DMA((G,)),
            pltpu.SemaphoreType.DMA((G,)),
            pltpu.SemaphoreType.DMA((4,)),
            pltpu.SemaphoreType.DMA((1,)),
            pltpu.SemaphoreType.DMA((1,)),
            pltpu.SemaphoreType.DMA((4,)),
        ],
        compiler_params=pltpu.CompilerParams(vmem_limit_bytes=110 * 1024 * 1024),
    )(
        A_x.reshape(B, D), A_k_cache, A_v_cache, A_wq, A_wo, B_w1,
        B_b1.reshape(1, F), B_w2, B_b2.reshape(1, D), grad_out.reshape(B, D),
    )
    out, gx, gk, gv, gwq, gwo, gw1, gb1, gw2, gb2 = outs
    return (out.reshape(B, Sq, D), gx.reshape(B, Sq, D), gk, gv, gwq, gwo,
            gw1, gb1.reshape(F), gw2, gb2.reshape(D))
```

```python
import math

import jax
import jax.numpy as jnp
from jax import lax
import jax.experimental.pallas as pl
import jax.experimental.pallas.tpu as pltpu

_F32 = jnp.float32
_BF16 = jnp.bfloat16
_NT = (((1,), (1,)), ((), ()))


def _dot(a, b):
    return jnp.dot(a, b, preferred_element_type=_F32)


def _dot_nt(a, b):
    return lax.dot_general(a, b, _NT, preferred_element_type=_F32)


def _ln_fwd(x):
    m = jnp.mean(x, axis=-1, keepdims=True)
    xc = x - m
    var = jnp.mean(xc * xc, axis=-1, keepdims=True)
    rstd = lax.rsqrt(var + 1e-5)
    return xc * rstd, rstd


def _ln_bwd(dxn, xn, rstd):
    m1 = jnp.mean(dxn, axis=-1, keepdims=True)
    m2 = jnp.mean(dxn * xn, axis=-1, keepdims=True)
    return rstd * (dxn - m1 - xn * m2)


_GELU_C = math.sqrt(2.0 / math.pi)


def _gelu_and_grad(x):
    x2 = x * x
    t = jnp.tanh(_GELU_C * (x + 0.044715 * x2 * x))
    y = 0.5 * x * (1.0 + t)
    dy = 0.5 * (1.0 + t) + 0.5 * x * (1.0 - t * t) * _GELU_C * (1.0 + 3.0 * 0.044715 * x2)
    return y, dy


@jax.jit
def pallas_interleave_layers__sliding_block_cached__dense_activation_gelu__decode_kernel(
    A_x: jax.Array,
    A_k_cache: jax.Array,
    A_v_cache: jax.Array,
    A_wq: jax.Array,
    A_wo: jax.Array,
    B_x: jax.Array,
    B_w1: jax.Array,
    B_b1: jax.Array,
    B_w2: jax.Array,
    B_b2: jax.Array,
    grad_out: jax.Array,
):
    B, Sq, D = A_x.shape
    _, Hkv, Sk, Dh = A_k_cache.shape
    HD = A_wq.shape[1]
    Hq = HD // Dh
    F = B_w1.shape[1]
    W = min(4096, max(256, Sk // 4))
    rep = Hq // Hkv
    assert Sq == 1 and B == 2 and rep == 4 and Dh == 128 and Hq == 32
    G = B * Hkv
    R = G * 8
    assert R == 128
    NT = 16
    SR = Sk // NT
    NW = W // SR
    NZ = NT - NW
    CR = 64
    assert NW * SR == W and SR % CR == 0
    scale = Dh ** -0.5

    def kernel(x_ref, k_hbm, v_hbm, wq_hbm, wo_hbm, w1_hbm, b1_ref, w2_hbm, b2_ref, go_ref,
               out_ref, gx_ref, gk_hbm, gv_hbm, gwq_hbm, gwo_hbm, gw1_hbm, gb1_ref, gw2_hbm, gb2_ref,
               kb, vb, wq_v, wo_v, w1_v, w2_v, gwq_v, gwo_v, gw1_v, gw2_v, z_ref,
               p_all, ds_all, pt_ref, dst_ref, q_all, o_all, do_all, dq_all,
               row_ref, flat_ref,
               xa_p, dq_p, o_p, ga_p, xb_p, dh_p, h_p, gb_p,
               ksem, vsem, wsem, zsem, osem, gsem):
        def k_load(g):
            return pltpu.make_async_copy(k_hbm.at[g, NZ:NT], kb.at[g], ksem.at[g])

        def v_load(g):
            return pltpu.make_async_copy(v_hbm.at[g, NZ:NT], vb.at[g], vsem.at[g])

        w_loads = [
            pltpu.make_async_copy(wq_hbm, wq_v, wsem.at[0]),
            pltpu.make_async_copy(wo_hbm, wo_v, wsem.at[1]),
            pltpu.make_async_copy(w1_hbm, w1_v, wsem.at[2]),
            pltpu.make_async_copy(w2_hbm, w2_v, wsem.at[3]),
        ]
        w_loads[0].start()
        for g in range(G):
            k_load(g).start()
        for g in range(G):
            v_load(g).start()
        w_loads[1].start()
        w_loads[2].start()
        w_loads[3].start()

        q_all[...] = jnp.zeros(q_all.shape, _F32)
        do_all[...] = jnp.zeros(do_all.shape, _F32)
        for r in (xa_p, o_p, xb_p, h_p):
            r[...] = jnp.zeros(r.shape, r.dtype)
        for r in (dq_p, ga_p, dh_p, gb_p):
            r[...] = jnp.zeros(r.shape, r.dtype)

        def pad8(ref_2d):
            row_ref[...] = jnp.zeros(row_ref.shape, _F32)
            row_ref[0:B, :] = ref_2d[...].astype(_F32)
            return row_ref[...]

        def flat_to_rows(flat, tbl, layer):
            flat_ref[...] = flat
            for b in range(B):
                for h in range(Hq):
                    r = (b * Hkv + h // rep) * 8 + layer * rep + h % rep
                    tbl[r:r + 1, :] = flat_ref[b:b + 1, h * Dh:(h + 1) * Dh]

        def rows_to_flat(tbl, layer):
            flat_ref[...] = jnp.zeros(flat_ref.shape, _F32)
            for b in range(B):
                for h in range(Hq):
                    r = (b * Hkv + h // rep) * 8 + layer * rep + h % rep
                    flat_ref[b:b + 1, h * Dh:(h + 1) * Dh] = tbl[r:r + 1, :]
            return flat_ref[...]

        def attn_fwd(x, layer):
            xn, rstd = _ln_fwd(x)
            xa_p[layer * B:(layer + 1) * B, :] = xn[0:B, :]
            q = _dot(xn.astype(_BF16), wq_v[...])
            flat_to_rows(q.astype(_BF16).astype(_F32), q_all, layer)

            def body(g, c):
                r0 = pl.multiple_of(g * 8, 8)
                qg = q_all[pl.ds(r0, 8), :].astype(_BF16)
                s = _dot_nt(qg, kb[g].reshape(W, Dh)) * scale
                m = jnp.max(s, axis=-1, keepdims=True)
                e = jnp.exp(s - m)
                p = e / jnp.sum(e, axis=-1, keepdims=True)
                p_all[pl.ds(r0, 8), :] = p
                o_all[pl.ds(r0, 8), :] = _dot(p.astype(_BF16), vb[g].reshape(W, Dh))
                return c

            lax.fori_loop(0, G, body, 0)
            o = rows_to_flat(o_all, layer)
            o_p[layer * B:(layer + 1) * B, :] = o[0:B, :]
            y = _dot(o.astype(_BF16), wo_v[...])
            return x + y, xn, rstd

        def attn_bwd(gy, layer, xn, rstd):
            gyb = gy.astype(_BF16)
            ga_p[layer * B:(layer + 1) * B, :] = gyb[0:B, :]
            do = _dot_nt(gyb, wo_v[...])
            flat_to_rows(do, do_all, layer)

            def body(g, c):
                r0 = pl.multiple_of(g * 8, 8)
                dog = do_all[pl.ds(r0, 8), :].astype(_BF16)
                dp = _dot_nt(dog, vb[g].reshape(W, Dh))
                p = p_all[pl.ds(r0, 8), :]
                ds = p * (dp - jnp.sum(p * dp, axis=-1, keepdims=True)) * scale
                ds_all[pl.ds(r0, 8), :] = ds
                dq_all[pl.ds(r0, 8), :] = _dot(ds.astype(_BF16), kb[g].reshape(W, Dh))
                return c

            lax.fori_loop(0, G, body, 0)
            dq = rows_to_flat(dq_all, layer).astype(_BF16)
            dq_p[layer * B:(layer + 1) * B, :] = dq[0:B, :]
            dxn = _dot_nt(dq, wq_v[...])
            return gy + _ln_bwd(dxn, xn, rstd)

        def ffn_fwd(x, layer):
            xn, rstd = _ln_fwd(x)
            xb_p[layer * B:(layer + 1) * B, :] = xn[0:B, :]
            hpre = _dot(xn.astype(_BF16), w1_v[...]) + b1_ref[...].astype(_F32).reshape(1, F)
            h, dgelu = _gelu_and_grad(hpre)
            h_p[layer * B:(layer + 1) * B, :] = h[0:B, :]
            y = _dot(h.astype(_BF16), w2_v[...]) + b2_ref[...].astype(_F32).reshape(1, D)
            return x + y, xn, rstd, dgelu

        def ffn_bwd(gy, layer, xn, rstd, dgelu):
            gyb = gy.astype(_BF16)
            gb_p[layer * B:(layer + 1) * B, :] = gyb[0:B, :]
            dh = _dot_nt(gyb, w2_v[...])
            dhpre = dh * dgelu
            dhb = dhpre.astype(_BF16)
            dh_p[layer * B:(layer + 1) * B, :] = dhb[0:B, :]
            dxn = _dot_nt(dhb, w1_v[...])
            db1 = jnp.sum(dhpre[0:B, :], axis=0, keepdims=True)
            db2 = jnp.sum(gy[0:B, :], axis=0, keepdims=True)
            return gy + _ln_bwd(dxn, xn, rstd), db1, db2

        z_ref[...] = jnp.zeros(z_ref.shape, z_ref.dtype)
        w_loads[0].wait()
        for g in range(G):
            k_load(g).wait()
        for g in range(G):
            v_load(g).wait()
        w_loads[1].wait()
        w_loads[2].wait()
        w_loads[3].wait()
        z_copies = []
        for c in range(SR // CR):
            for dst in (gk_hbm, gv_hbm):
                cp = pltpu.make_async_copy(
                    z_ref, dst.at[:, 0:NZ, pl.ds(c * CR, CR), :], zsem.at[0])
                cp.start()
                z_copies.append(cp)

        x0 = pad8(x_ref)
        x1, xn_a0, rs_a0 = attn_fwd(x0, 0)
        x2, xn_b0, rs_b0, dg0 = ffn_fwd(x1, 0)
        x3, xn_a1, rs_a1 = attn_fwd(x2, 1)
        x4, xn_b1, rs_b1, dg1 = ffn_fwd(x3, 1)
        out_ref[...] = x4[0:B, :].astype(out_ref.dtype)

        g4 = pad8(go_ref)
        g3, db1_1, db2_1 = ffn_bwd(g4, 1, xn_b1, rs_b1, dg1)
        g2 = attn_bwd(g3, 1, xn_a1, rs_a1)
        g1, db1_0, db2_0 = ffn_bwd(g2, 0, xn_b0, rs_b0, dg0)
        g0 = attn_bwd(g1, 0, xn_a0, rs_a0)
        gx_ref[...] = g0[0:B, :].astype(gx_ref.dtype)
        gb1_ref[...] = (db1_0 + db1_1).reshape(F).astype(gb1_ref.dtype)
        gb2_ref[...] = (db2_0 + db2_1).reshape(D).astype(gb2_ref.dtype)

        out_copies = []
        for i, (lhs, rhs, stage, dst) in enumerate((
                (xa_p, dq_p, gwq_v, gwq_hbm), (o_p, ga_p, gwo_v, gwo_hbm),
                (xb_p, dh_p, gw1_v, gw1_hbm), (h_p, gb_p, gw2_v, gw2_hbm))):
            lt = lhs[...].T.astype(_BF16)
            stage[...] = _dot(lt, rhs[...]).astype(_BF16)
            cp = pltpu.make_async_copy(stage, dst, gsem.at[i])
            cp.start()
            out_copies.append(cp)

        pt_ref[...] = p_all[...].T.astype(_BF16)
        dst_ref[...] = ds_all[...].T.astype(_BF16)
        rgrp = lax.broadcasted_iota(jnp.int32, (R, Dh), 0) // 8
        qv = q_all[...]
        dov = do_all[...]
        for g in range(G):
            qm = jnp.where(rgrp == g, qv, 0.0).astype(_BF16)
            kb[g] = _dot(dst_ref[...], qm).astype(_BF16).reshape(NW, SR, Dh)
            dm = jnp.where(rgrp == g, dov, 0.0).astype(_BF16)
            vb[g] = _dot(pt_ref[...], dm).astype(_BF16).reshape(NW, SR, Dh)
        for c in range(SR // CR):
            for src, dst in ((kb, gk_hbm), (vb, gv_hbm)):
                cp = pltpu.make_async_copy(
                    src.at[:, :, pl.ds(c * CR, CR), :],
                    dst.at[:, NZ:NT, pl.ds(c * CR, CR), :], osem.at[0])
                cp.start()
                out_copies.append(cp)

        for cp in z_copies:
            cp.wait()
        for cp in out_copies:
            cp.wait()

    vmem = pl.BlockSpec(memory_space=pltpu.VMEM)
    hbm = pl.BlockSpec(memory_space=pl.ANY)
    outs = pl.pallas_call(
        kernel,
        in_specs=[vmem, hbm, hbm, hbm, hbm, hbm, vmem, hbm, vmem, vmem],
        out_specs=[vmem, vmem, hbm, hbm, hbm, hbm, hbm, vmem, hbm, vmem],
        out_shape=[
            jax.ShapeDtypeStruct((B, D), _BF16),
            jax.ShapeDtypeStruct((B, D), _BF16),
            jax.ShapeDtypeStruct((G, NT, SR, Dh), _BF16),
            jax.ShapeDtypeStruct((G, NT, SR, Dh), _BF16),
            jax.ShapeDtypeStruct(A_wq.shape, _BF16),
            jax.ShapeDtypeStruct(A_wo.shape, _BF16),
            jax.ShapeDtypeStruct(B_w1.shape, _BF16),
            jax.ShapeDtypeStruct((F,), _BF16),
            jax.ShapeDtypeStruct(B_w2.shape, _BF16),
            jax.ShapeDtypeStruct((D,), _BF16),
        ],
        scratch_shapes=[
            pltpu.VMEM((G, NW, SR, Dh), _BF16),
            pltpu.VMEM((G, NW, SR, Dh), _BF16),
            pltpu.VMEM((D, HD), _BF16),
            pltpu.VMEM((HD, D), _BF16),
            pltpu.VMEM((D, F), _BF16),
            pltpu.VMEM((F, D), _BF16),
            pltpu.VMEM((D, HD), _BF16),
            pltpu.VMEM((HD, D), _BF16),
            pltpu.VMEM((D, F), _BF16),
            pltpu.VMEM((F, D), _BF16),
            pltpu.VMEM((G, NZ, CR, Dh), _BF16),
            pltpu.VMEM((R, W), _F32),
            pltpu.VMEM((R, W), _F32),
            pltpu.VMEM((W, R), _BF16),
            pltpu.VMEM((W, R), _BF16),
            pltpu.VMEM((R, Dh), _F32),
            pltpu.VMEM((R, Dh), _F32),
            pltpu.VMEM((R, Dh), _F32),
            pltpu.VMEM((R, Dh), _F32),
            pltpu.VMEM((8, D), _F32),
            pltpu.VMEM((8, HD), _F32),
            pltpu.VMEM((128, D), _F32),
            pltpu.VMEM((128, HD), _BF16),
            pltpu.VMEM((128, HD), _F32),
            pltpu.VMEM((128, D), _BF16),
            pltpu.VMEM((128, D), _F32),
            pltpu.VMEM((128, F), _BF16),
            pltpu.VMEM((128, F), _F32),
            pltpu.VMEM((128, D), _BF16),
            pltpu.SemaphoreType.DMA((G,)),
            pltpu.SemaphoreType.DMA((G,)),
            pltpu.SemaphoreType.DMA((4,)),
            pltpu.SemaphoreType.DMA((1,)),
            pltpu.SemaphoreType.DMA((1,)),
            pltpu.SemaphoreType.DMA((4,)),
        ],
        compiler_params=pltpu.CompilerParams(vmem_limit_bytes=110 * 1024 * 1024),
    )(
        A_x.reshape(B, D), A_k_cache.reshape(G, NT, SR, Dh), A_v_cache.reshape(G, NT, SR, Dh), A_wq, A_wo, B_w1,
        B_b1, B_w2, B_b2, grad_out.reshape(B, D),
    )
    out, gx, gk, gv, gwq, gwo, gw1, gb1, gw2, gb2 = outs
    return (out.reshape(B, Sq, D), gx.reshape(B, Sq, D), gk.reshape(A_k_cache.shape),
            gv.reshape(A_v_cache.shape), gwq, gwo,
            gw1, gb1, gw2, gb2)
```

```python
import math

import jax
import jax.numpy as jnp
from jax import lax
import jax.experimental.pallas as pl
import jax.experimental.pallas.tpu as pltpu

_F32 = jnp.float32
_BF16 = jnp.bfloat16
_NT_DIMS = (((1,), (1,)), ((), ()))


def _dot(a, b):
    return jnp.dot(a, b, preferred_element_type=_F32)


def _dot_nt(a, b):
    return lax.dot_general(a, b, _NT_DIMS, preferred_element_type=_F32)


def _ln_fwd(x):
    m = jnp.mean(x, axis=-1, keepdims=True)
    xc = x - m
    var = jnp.mean(xc * xc, axis=-1, keepdims=True)
    rstd = lax.rsqrt(var + 1e-5)
    return xc * rstd, rstd


def _ln_bwd(dxn, xn, rstd):
    m1 = jnp.mean(dxn, axis=-1, keepdims=True)
    m2 = jnp.mean(dxn * xn, axis=-1, keepdims=True)
    return rstd * (dxn - m1 - xn * m2)


_GELU_C = math.sqrt(2.0 / math.pi)


def _gelu_and_grad(x):
    x2 = x * x
    t = jnp.tanh(_GELU_C * (x + 0.044715 * x2 * x))
    y = 0.5 * x * (1.0 + t)
    dy = 0.5 * (1.0 + t) + 0.5 * x * (1.0 - t * t) * _GELU_C * (1.0 + 3.0 * 0.044715 * x2)
    return y, dy


@jax.jit
def pallas_interleave_layers__sliding_block_cached__dense_activation_gelu__decode_kernel(
    A_x: jax.Array,
    A_k_cache: jax.Array,
    A_v_cache: jax.Array,
    A_wq: jax.Array,
    A_wo: jax.Array,
    B_x: jax.Array,
    B_w1: jax.Array,
    B_b1: jax.Array,
    B_w2: jax.Array,
    B_b2: jax.Array,
    grad_out: jax.Array,
):
    B, Sq, D = A_x.shape
    _, Hkv, Sk, Dh = A_k_cache.shape
    HD = A_wq.shape[1]
    Hq = HD // Dh
    F = B_w1.shape[1]
    W = min(4096, max(256, Sk // 4))
    rep = Hq // Hkv
    assert Sq == 1 and B == 2 and rep == 4 and Dh == 128 and Hq == 32
    G = B * Hkv
    R = G * 8
    assert R == 128
    scale = Dh ** -0.5

    NT = 16
    SR = Sk // NT
    NW = W // SR
    NZ = NT - NW
    ZR = 64
    WR = 128
    assert NW * SR == W and SR % ZR == 0 and SR % WR == 0
    gwq_view, gwq_seg = (8, D // 8, HD), (16, HD // 4)
    gwo_view, gwo_seg = (8, HD // 8, D), (32, D)
    gw1_view, gw1_seg = (4, D // 4, F), (16, F // 2)
    gw2_view, gw2_seg = (4, F // 4, D), (32, D)

    def kernel(x_hbm, k_hbm, v_hbm, wq_hbm, wo_hbm, w1_hbm, b1_hbm, w2_hbm, b2_hbm, go_hbm,
               out_hbm, gx_hbm, gk_hbm, gv_hbm, gwq_hbm, gwo_hbm, gw1_hbm, gb1_hbm, gw2_hbm,
               gb2_hbm,
               x_ref, b1_ref, b2_ref, go_ref, out_ref, gx_ref, gb1_ref, gb2_ref,
               kb, vb, wq_v, wo_v, w1_v, w2_v, gwq_v, gwo_v, gw1_v, gw2_v, z_ref,
               p_all, ds_all, pt_ref, dst_ref, q_all, o_all, do_all, dq_all,
               row_ref, flat_ref,
               xa_p, dq_p, o_p, ga_p, xb_p, dh_p, h_p, gb_p,
               ssem, ksem, vsem, wsem, zsem, osem, gsem):
        loads = [pltpu.make_async_copy(a, b, ssem.at[i]) for i, (a, b) in enumerate(
            ((x_hbm, x_ref), (b1_hbm, b1_ref), (b2_hbm, b2_ref), (go_hbm, go_ref)))]
        loads.append(pltpu.make_async_copy(wq_hbm, wq_v, wsem.at[0]))
        loads += [pltpu.make_async_copy(k_hbm.at[g, NZ:NT], kb.at[g], ksem.at[g])
                  for g in range(G)]
        loads += [pltpu.make_async_copy(v_hbm.at[g, NZ:NT], vb.at[g], vsem.at[g])
                  for g in range(G)]
        loads.append(pltpu.make_async_copy(wo_hbm, wo_v, wsem.at[1]))
        loads.append(pltpu.make_async_copy(w1_hbm, w1_v, wsem.at[2]))
        loads.append(pltpu.make_async_copy(w2_hbm, w2_v, wsem.at[3]))
        for cp in loads:
            cp.start()

        for r in (q_all, do_all, xa_p, dq_p, o_p, ga_p, xb_p, dh_p, h_p, gb_p, z_ref):
            r[...] = jnp.zeros(r.shape, r.dtype)

        for cp in loads:
            cp.wait()
        writes = []
        for c in range(SR // ZR):
            for dst in (gk_hbm, gv_hbm):
                cp = pltpu.make_async_copy(
                    z_ref, dst.at[:, 0:NZ, pl.ds(c * ZR, ZR), :], zsem.at[0])
                cp.start()
                writes.append(cp)

        def pad8(ref_2d):
            row_ref[...] = jnp.zeros(row_ref.shape, _F32)
            row_ref[0:B, :] = ref_2d[...].astype(_F32)
            return row_ref[...]

        def tbl_row(b, h, layer):
            return (b * Hkv + h // rep) * 8 + layer * rep + h % rep

        def flat_to_rows(flat, tbl, layer):
            flat_ref[...] = flat
            for b in range(B):
                for h in range(Hq):
                    r = tbl_row(b, h, layer)
                    tbl[r:r + 1, :] = flat_ref[b:b + 1, h * Dh:(h + 1) * Dh]

        def rows_to_flat(tbl, layer):
            flat_ref[...] = jnp.zeros(flat_ref.shape, _F32)
            for b in range(B):
                for h in range(Hq):
                    r = tbl_row(b, h, layer)
                    flat_ref[b:b + 1, h * Dh:(h + 1) * Dh] = tbl[r:r + 1, :]
            return flat_ref[...]

        def attn_fwd(x, layer):
            xn, rstd = _ln_fwd(x)
            xa_p[layer * B:(layer + 1) * B, :] = xn[0:B, :]
            q = _dot(xn.astype(_BF16), wq_v[...])
            flat_to_rows(q.astype(_BF16).astype(_F32), q_all, layer)

            def body(g, c):
                r0 = pl.multiple_of(g * 8, 8)
                qg = q_all[pl.ds(r0, 8), :].astype(_BF16)
                s = _dot_nt(qg, kb[g].reshape(W, Dh)) * scale
                m = jnp.max(s, axis=-1, keepdims=True)
                e = jnp.exp(s - m)
                p = e / jnp.sum(e, axis=-1, keepdims=True)
                p_all[pl.ds(r0, 8), :] = p
                o_all[pl.ds(r0, 8), :] = _dot(p.astype(_BF16), vb[g].reshape(W, Dh))
                return c

            lax.fori_loop(0, G, body, 0)
            o = rows_to_flat(o_all, layer)
            o_p[layer * B:(layer + 1) * B, :] = o[0:B, :]
            y = _dot(o.astype(_BF16), wo_v[...])
            return x + y, xn, rstd

        def attn_bwd(gy, layer, xn, rstd):
            gyb = gy.astype(_BF16)
            ga_p[layer * B:(layer + 1) * B, :] = gyb[0:B, :]
            do = _dot_nt(gyb, wo_v[...])
            flat_to_rows(do, do_all, layer)

            def body(g, c):
                r0 = pl.multiple_of(g * 8, 8)
                dog = do_all[pl.ds(r0, 8), :].astype(_BF16)
                dp = _dot_nt(dog, vb[g].reshape(W, Dh))
                p = p_all[pl.ds(r0, 8), :]
                ds = p * (dp - jnp.sum(p * dp, axis=-1, keepdims=True)) * scale
                ds_all[pl.ds(r0, 8), :] = ds
                dq_all[pl.ds(r0, 8), :] = _dot(ds.astype(_BF16), kb[g].reshape(W, Dh))
                return c

            lax.fori_loop(0, G, body, 0)
            dq = rows_to_flat(dq_all, layer).astype(_BF16)
            dq_p[layer * B:(layer + 1) * B, :] = dq[0:B, :]
            dxn = _dot_nt(dq, wq_v[...])
            return gy + _ln_bwd(dxn, xn, rstd)

        def ffn_fwd(x, layer):
            xn, rstd = _ln_fwd(x)
            xb_p[layer * B:(layer + 1) * B, :] = xn[0:B, :]
            hpre = _dot(xn.astype(_BF16), w1_v[...]) + b1_ref[...].astype(_F32).reshape(1, F)
            h, dgelu = _gelu_and_grad(hpre)
            h_p[layer * B:(layer + 1) * B, :] = h[0:B, :]
            y = _dot(h.astype(_BF16), w2_v[...]) + b2_ref[...].astype(_F32).reshape(1, D)
            return x + y, xn, rstd, dgelu

        def ffn_bwd(gy, layer, xn, rstd, dgelu):
            gyb = gy.astype(_BF16)
            gb_p[layer * B:(layer + 1) * B, :] = gyb[0:B, :]
            dh = _dot_nt(gyb, w2_v[...])
            dhpre = dh * dgelu
            dhb = dhpre.astype(_BF16)
            dh_p[layer * B:(layer + 1) * B, :] = dhb[0:B, :]
            dxn = _dot_nt(dhb, w1_v[...])
            db1 = jnp.sum(dhpre[0:B, :], axis=0, keepdims=True)
            db2 = jnp.sum(gy[0:B, :], axis=0, keepdims=True)
            return gy + _ln_bwd(dxn, xn, rstd), db1, db2

        x0 = pad8(x_ref)
        x1, xn_a0, rs_a0 = attn_fwd(x0, 0)
        x2, xn_b0, rs_b0, dg0 = ffn_fwd(x1, 0)
        x3, xn_a1, rs_a1 = attn_fwd(x2, 1)
        x4, xn_b1, rs_b1, dg1 = ffn_fwd(x3, 1)
        out_ref[...] = x4[0:B, :].astype(out_ref.dtype)

        g4 = pad8(go_ref)
        g3, db1_1, db2_1 = ffn_bwd(g4, 1, xn_b1, rs_b1, dg1)
        g2 = attn_bwd(g3, 1, xn_a1, rs_a1)
        g1, db1_0, db2_0 = ffn_bwd(g2, 0, xn_b0, rs_b0, dg0)
        g0 = attn_bwd(g1, 0, xn_a0, rs_a0)
        gx_ref[...] = g0[0:B, :].astype(gx_ref.dtype)
        gb1_ref[...] = (db1_0 + db1_1).reshape(F).astype(gb1_ref.dtype)
        gb2_ref[...] = (db2_0 + db2_1).reshape(D).astype(gb2_ref.dtype)
        for i, (a, b) in enumerate(((out_ref, out_hbm), (gx_ref, gx_hbm),
                                    (gb1_ref, gb1_hbm), (gb2_ref, gb2_hbm))):
            cp = pltpu.make_async_copy(a, b, ssem.at[4 + i])
            cp.start()
            writes.append(cp)

        w_jobs = []
        for lhs, rhs, stage, dst, (rb, cb) in (
                (xa_p, dq_p, gwq_v, gwq_hbm, gwq_seg), (o_p, ga_p, gwo_v, gwo_hbm, gwo_seg),
                (xb_p, dh_p, gw1_v, gw1_hbm, gw1_seg), (h_p, gb_p, gw2_v, gw2_hbm, gw2_seg)):
            lt = lhs[...].T.astype(_BF16)
            stage[...] = _dot(lt, rhs[...]).astype(_BF16).reshape(stage.shape)
            w_jobs.append([(stage, dst, r, c, rb, cb)
                           for r in range(0, stage.shape[1], rb)
                           for c in range(0, stage.shape[2], cb)])
        for j in range(max(len(t) for t in w_jobs)):
            for t in w_jobs:
                if j < len(t):
                    stage, dst, r, c, rb, cb = t[j]
                    cp = pltpu.make_async_copy(
                        stage.at[:, r:r + rb, c:c + cb], dst.at[:, r:r + rb, c:c + cb],
                        gsem.at[0])
                    cp.start()
                    writes.append(cp)

        pt_ref[...] = p_all[...].T.astype(_BF16)
        dst_ref[...] = ds_all[...].T.astype(_BF16)
        rgrp = lax.broadcasted_iota(jnp.int32, (R, Dh), 0) // 8
        qv = q_all[...]
        dov = do_all[...]
        for g in range(G):
            qm = jnp.where(rgrp == g, qv, 0.0).astype(_BF16)
            kb[g] = _dot(dst_ref[...], qm).astype(_BF16).reshape(NW, SR, Dh)
            dm = jnp.where(rgrp == g, dov, 0.0).astype(_BF16)
            vb[g] = _dot(pt_ref[...], dm).astype(_BF16).reshape(NW, SR, Dh)
        for c in range(SR // WR):
            for src, dst in ((kb, gk_hbm), (vb, gv_hbm)):
                cp = pltpu.make_async_copy(
                    src.at[:, :, pl.ds(c * WR, WR), :],
                    dst.at[:, NZ:NT, pl.ds(c * WR, WR), :], osem.at[0])
                cp.start()
                writes.append(cp)

        for cp in writes:
            cp.wait()

    hbm = pl.BlockSpec(memory_space=pl.ANY)
    outs = pl.pallas_call(
        kernel,
        in_specs=[hbm] * 10,
        out_specs=[hbm] * 10,
        out_shape=[
            jax.ShapeDtypeStruct((B, D), _BF16),
            jax.ShapeDtypeStruct((B, D), _BF16),
            jax.ShapeDtypeStruct((G, NT, SR, Dh), _BF16),
            jax.ShapeDtypeStruct((G, NT, SR, Dh), _BF16),
            jax.ShapeDtypeStruct(gwq_view, _BF16),
            jax.ShapeDtypeStruct(gwo_view, _BF16),
            jax.ShapeDtypeStruct(gw1_view, _BF16),
            jax.ShapeDtypeStruct((F,), _BF16),
            jax.ShapeDtypeStruct(gw2_view, _BF16),
            jax.ShapeDtypeStruct((D,), _BF16),
        ],
        scratch_shapes=[
            pltpu.VMEM((B, D), _BF16),
            pltpu.VMEM((F,), _BF16),
            pltpu.VMEM((D,), _BF16),
            pltpu.VMEM((B, D), _BF16),
            pltpu.VMEM((B, D), _BF16),
            pltpu.VMEM((B, D), _BF16),
            pltpu.VMEM((F,), _BF16),
            pltpu.VMEM((D,), _BF16),
            pltpu.VMEM((G, NW, SR, Dh), _BF16),
            pltpu.VMEM((G, NW, SR, Dh), _BF16),
            pltpu.VMEM((D, HD), _BF16),
            pltpu.VMEM((HD, D), _BF16),
            pltpu.VMEM((D, F), _BF16),
            pltpu.VMEM((F, D), _BF16),
            pltpu.VMEM(gwq_view, _BF16),
            pltpu.VMEM(gwo_view, _BF16),
            pltpu.VMEM(gw1_view, _BF16),
            pltpu.VMEM(gw2_view, _BF16),
            pltpu.VMEM((G, NZ, ZR, Dh), _BF16),
            pltpu.VMEM((R, W), _F32),
            pltpu.VMEM((R, W), _F32),
            pltpu.VMEM((W, R), _BF16),
            pltpu.VMEM((W, R), _BF16),
            pltpu.VMEM((R, Dh), _F32),
            pltpu.VMEM((R, Dh), _F32),
            pltpu.VMEM((R, Dh), _F32),
            pltpu.VMEM((R, Dh), _F32),
            pltpu.VMEM((8, D), _F32),
            pltpu.VMEM((8, HD), _F32),
            pltpu.VMEM((128, D), _F32),
            pltpu.VMEM((128, HD), _BF16),
            pltpu.VMEM((128, HD), _F32),
            pltpu.VMEM((128, D), _BF16),
            pltpu.VMEM((128, D), _F32),
            pltpu.VMEM((128, F), _BF16),
            pltpu.VMEM((128, F), _F32),
            pltpu.VMEM((128, D), _BF16),
            pltpu.SemaphoreType.DMA((8,)),
            pltpu.SemaphoreType.DMA((G,)),
            pltpu.SemaphoreType.DMA((G,)),
            pltpu.SemaphoreType.DMA((4,)),
            pltpu.SemaphoreType.DMA((1,)),
            pltpu.SemaphoreType.DMA((1,)),
            pltpu.SemaphoreType.DMA((1,)),
        ],
        compiler_params=pltpu.CompilerParams(vmem_limit_bytes=110 * 1024 * 1024),
    )(
        A_x.reshape(B, D), A_k_cache.reshape(G, NT, SR, Dh), A_v_cache.reshape(G, NT, SR, Dh),
        A_wq, A_wo, B_w1, B_b1, B_w2, B_b2, grad_out.reshape(B, D),
    )
    out, gx, gk, gv, gwq, gwo, gw1, gb1, gw2, gb2 = outs
    return (out.reshape(B, Sq, D), gx.reshape(B, Sq, D),
            gk.reshape(A_k_cache.shape), gv.reshape(A_v_cache.shape),
            gwq.reshape(A_wq.shape), gwo.reshape(A_wo.shape),
            gw1.reshape(B_w1.shape), gb1, gw2.reshape(B_w2.shape), gb2)
```
